```python
import os as _os
_os.environ.setdefault("JAX_PLATFORMS", "cpu")
import jax
import jax.numpy as jnp

def _softmax(x, axis=-1):
    return jax.nn.softmax(x, axis=axis)
def _gelu(x):
    return jax.nn.gelu(x, approximate=True)
def _silu(x):
    return jax.nn.silu(x)
def _sigmoid(x):
    return jax.nn.sigmoid(x)
def _layernorm(x, axis=-1, eps=1e-5):
    m = jnp.mean(x, axis=axis, keepdims=True)
    v = jnp.var(x, axis=axis, keepdims=True)
    return (x - m) / jnp.sqrt(v + eps)
def _scatter_add(tgt, idx, src, axis=0):
    return tgt.at[idx].add(src)
def _segment_sum(src, seg, n):
    return jax.ops.segment_sum(src, seg, n)
class _Rng:
    def __init__(self, key):
        self._k = key
    def _next(self):
        self._k, sub = jax.random.split(self._k)
        return sub
    def normal(self, shape):
        return jax.random.normal(self._next(), shape, dtype=jnp.bfloat16)
    def randint(self, lo, hi, shape):
        return jax.random.randint(self._next(), shape, lo, hi, dtype=jnp.int32)
    def uniform(self, shape, lo=0.0, hi=1.0):
        return jax.random.uniform(self._next(), shape, jnp.bfloat16, lo, hi)
    def permutation(self, n):
        return jax.random.permutation(self._next(), n)


kernel_name = 'sequential_preLN__ssm_conv_h3__mixer_s_mlp__prompt'

def setup_inputs():
    _rng = _Rng(jax.random.key(int.from_bytes(__import__("os").urandom(4), "little")))
    _w = (lambda a: (lambda t: t.astype(jnp.bfloat16) if jnp.issubdtype(t.dtype, jnp.floating) else t)(jnp.asarray(a)))
    def _A_setup():
        B, S, D = 1, 2048, 640
        ks = 4
        return {
            "q": _w((lambda *s: _rng.normal(s) * 0.05)(B, S, D)),
            "k": _w((lambda *s: _rng.normal(s) * 0.05)(B, S, D)),
            "v": _w((lambda *s: _rng.normal(s) * 0.05)(B, S, D)),
            "shift_k": _w((lambda *s: _rng.normal(s) * 0.05)(D, ks) * 0.5),
            "ssm_k": _w((lambda *s: _rng.normal(s) * 0.05)(D, S) * (1.0 / S ** 0.5)),
            "ssm_D": _w((lambda *s: _rng.normal(s) * 0.05)(D)),
        }
    _A_in = _A_setup()

    def _B_setup():
        B, S, D, F = 1, 2048, 640, 1728
        return {
            "x":  _w((lambda *s: _rng.normal(s) * 0.05)(B, S, D)),
            "w1": _w((lambda *s: _rng.normal(s) * 0.8)(D, D) * (D ** -0.5)),
            "w2": _w((lambda *s: _rng.normal(s) * 0.8)(D, D) * (D ** -0.5)),
            "w3": _w((lambda *s: _rng.normal(s) * 0.8)(D, F) * (D ** -0.5)),
            "w4": _w((lambda *s: _rng.normal(s) * 0.8)(F, D) * (F ** -0.5)),
        }
    _B_in = _B_setup()

    return {
        "A_q": _A_in["q"],
        "A_k": _A_in["k"],
        "A_v": _A_in["v"],
        "A_shift_k": _A_in["shift_k"],
        "A_ssm_k": _A_in["ssm_k"],
        "A_ssm_D": _A_in["ssm_D"],
        "B_x": _B_in["x"],
        "B_w1": _B_in["w1"],
        "B_w2": _B_in["w2"],
        "B_w3": _B_in["w3"],
        "B_w4": _B_in["w4"],
    }

def reference(A_q, A_k, A_v, A_shift_k, A_ssm_k, A_ssm_D, B_x, B_w1, B_w2, B_w3, B_w4):
    def _A_ref(q, k, v, shift_k, ssm_k, ssm_D):
        B, S, D = q.shape
        ks = shift_k.shape[-1]
        k_pad = jnp.pad(k, ((0, 0), (ks - 1, 0), (0, 0)))
        k_shift = jnp.zeros_like(k)
        for t in range(ks):
            k_shift = k_shift + k_pad[:, t:t + S, :] * shift_k[:, ks - 1 - t][None, None, :]
        kv = k_shift * v
        L = 2 * S
        kv_pad = jnp.pad(kv, ((0, 0), (0, S), (0, 0)))
        kf_pad = jnp.pad(ssm_k, ((0, 0), (0, S)))
        kv_f = (lambda x, axes=(-2,-1): jnp.fft.rfft2(x.astype(jnp.float32), axes=axes))(kv_pad[:, None, :, :], axes=(1, 2))
        kf_f = (lambda x, axes=(-2,-1): jnp.fft.rfft2(x.astype(jnp.float32), axes=axes))(kf_pad[:, None, :], axes=(1, 2))
        kf_f = (lambda x, *d: x.transpose(*d))(kf_f, 1, 2, 0)
        y_f = kv_f * kf_f[None, :, :, :]
        y = (lambda x, s, axes=(-2,-1): jnp.fft.irfft2(x, s=s, axes=axes).astype(jnp.bfloat16))(y_f, (1, L), axes=(1, 2))[:, 0, :S, :]
        y = y + kv * ssm_D[None, None, :]
        return q * y

    def _B_ref(x, w1, w2, w3, w4):
        B, S, D = x.shape
        h = _gelu(_layernorm(x, axis=-1) @ w1)
        c = D // 4
        g0 = jnp.pad(h[:, :, 0*c:1*c], ((0, 0), (1, 0), (0, 0)))[:, :S, :]
        g1 = jnp.pad(h[:, :, 1*c:2*c], ((0, 0), (0, 1), (0, 0)))[:, 1:, :]
        g2 = jnp.pad(h[:, :, 2*c:3*c], ((0, 0), (2, 0), (0, 0)))[:, :S, :]
        g3 = jnp.pad(h[:, :, 3*c:   ], ((0, 0), (0, 2), (0, 0)))[:, 2:, :]
        hs = jnp.concatenate([g0, g1, g2, g3], axis=-1) @ w2
        x1 = x + hs
        h2 = _gelu(_layernorm(x1, axis=-1) @ w3) @ w4
        return x1 + h2

    x = A_q
    h = x + _A_ref(_layernorm(x, axis=-1), A_k, A_v, A_shift_k, A_ssm_k, A_ssm_D)
    h2 = h + _B_ref(_layernorm(h, axis=-1), B_w1, B_w2, B_w3, B_w4)
    return h2
```

```python
import jax
import jax.numpy as jnp
import numpy as np
import jax.experimental.pallas as pl
import jax.experimental.pallas.tpu as pltpu
from jax import lax

f32, bf16, u32, i32 = jnp.float32, jnp.bfloat16, jnp.uint32, jnp.int32

S, D, FF = 2048, 640, 1728
NT = D // 128
BLK = 512
NB = S // BLK
LFFT = 2 * BLK
PADW = 8
APAD = 8
EPS = 1e-5


def _bf16_bits(a):
    u = np.ascontiguousarray(a, dtype=np.float32).view(np.uint32).astype(np.uint64)
    r = (u + 0x7FFF + ((u >> 16) & 1)) >> 16
    return (r & 0xFFFF).astype(np.uint32)


def _pack_words(a):
    b = _bf16_bits(a)
    return (b[..., 0::2, :] | (b[..., 1::2, :] << np.uint32(16))).astype(np.uint32)


def _dft_constants():
    k1 = np.zeros((16, 8), np.int64)
    for v in range(16):
        for s in range(8):
            k1[v, s] = 2 * (8 * v + s) if v < 8 else 2 * (8 * (v - 8) + s) + 1
    n1 = np.arange(128)
    fm = np.zeros((4, 256, 128))
    gm = np.zeros((4, 128, 256))
    for r in range(4):
        for v in range(16):
            for s in range(8):
                th = 2 * np.pi * (4 * n1 + r) * (k1[v, s] + 0.5) / LFFT
                fm[r, 16 * v + s] = np.cos(th)
                fm[r, 16 * v + 8 + s] = -np.sin(th)
                gm[r, :, 16 * v + s] = np.cos(th) * (2.0 / LFFT)
                gm[r, :, 16 * v + 8 + s] = -np.sin(th) * (2.0 / LFFT)
    return _pack_words(fm), _pack_words(gm)


def _dot(a, b):
    return jnp.dot(a, b, preferred_element_type=f32)


def _dot_nt(a, b):
    return lax.dot_general(a, b, (((1,), (1,)), ((), ())), preferred_element_type=f32)


def _lo(w):
    return pltpu.bitcast(w << 16, f32)


def _hi(w):
    return pltpu.bitcast(w & jnp.uint32(0xFFFF0000), f32)


def _ln(x):
    m = jnp.mean(x, axis=-1, keepdims=True)
    d = x - m
    v = jnp.mean(d * d, axis=-1, keepdims=True)
    return d * lax.rsqrt(v + EPS)


C0 = float(np.sqrt(2.0 / np.pi))
C1 = float(np.sqrt(2.0 / np.pi) * 0.044715)


def _gelu(x):
    inner = x * (C0 + C1 * (x * x))
    hx = 0.5 * x
    return hx + hx * jnp.tanh(inner)


def _cat(xs):
    return jnp.concatenate(xs, axis=1)


def _kernel(x_hbm, k_hbm, v_hbm, sk_hbm, ssmk_hbm, d_hbm, w1_hbm, w2_hbm, w3_hbm, w4_hbm, f_hbm, g_hbm,
            o_hbm,
            KR, VR, XR, SK, W1, W2, W3, W4, FS, GS, SKS, DS, TAP, TB, UB, KB, U, KP, BB, H, XB, A, OUT, sems):
    nsem = [0]

    def dma(src, dst):
        i = nsem[0]
        nsem[0] += 1
        return pltpu.make_async_copy(src, dst, sems.at[i])

    def tiles(src, dst, r0, nrows, dr0=None):
        dr0 = r0 if dr0 is None else dr0
        return [dma(src.at[pl.ds(r0, nrows), pl.ds(128 * c, 128)], dst.at[c, pl.ds(dr0, nrows), :]) for c in range(NT)]

    cp = {}
    cp['small'] = [dma(sk_hbm, SKS), dma(d_hbm, DS)]
    cp['f'] = [dma(f_hbm, FS)]
    for j in range(NB):
        cp['sk', j] = [dma(ssmk_hbm.at[:, pl.ds(BLK * j, BLK)], SK.at[:, pl.ds(BLK * j, BLK)])]
        cp['k', j] = tiles(k_hbm, KR, BLK * j, BLK, 2 * PADW + BLK * j)
        cp['v', j] = tiles(v_hbm, VR, BLK * j, BLK)
        cp['x', j] = tiles(x_hbm, XR, BLK * j, BLK)
    cp['g'] = [dma(g_hbm, GS)]
    cp['w1'] = tiles(w1_hbm, W1, 0, D)
    cp['w2'] = tiles(w2_hbm, W2, 0, D)
    cp['w3'] = tiles(w3_hbm, W3, 0, FF)
    cp['w4'] = tiles(w4_hbm, W4, 0, FF)
    order = ['small', 'f', ('sk', 0), ('k', 0), ('v', 0), 'g', ('x', 0), 'w1', ('sk', 1), ('k', 1), ('v', 1), ('x', 1),
             'w2', 'w3', 'w4', ('sk', 2), ('k', 2), ('v', 2), ('x', 2), ('sk', 3), ('k', 3), ('v', 3), ('x', 3)]
    for key in order:
        for c in cp[key]:
            c.start()

    def wait(key):
        for c in cp[key]:
            c.wait()

    for c in range(NT):
        KR[c, pl.ds(0, 2 * PADW), :] = jnp.zeros((2 * PADW, 128), bf16)
        A[c, pl.ds(0, APAD), :] = jnp.zeros((APAD, 128), f32)
        A[c, pl.ds(APAD + S, APAD), :] = jnp.zeros((APAD, 128), f32)

    def wload(W, r0, nrows):
        return _cat([pltpu.bitcast(W.at[c].bitcast(u32)[pl.ds(r0 // 2, nrows // 2), :], bf16) for c in range(NT)])

    wait('small')
    skv = SKS[...].astype(f32)
    dv = DS[...].astype(f32).reshape(1, D)
    for t in range(4):
        for c in range(NT):
            TAP[t, c] = jnp.broadcast_to(skv[t:t + 1, 128 * c:128 * c + 128], (8, 128))
    for c in range(NT):
        TAP[4, c] = jnp.broadcast_to(dv[:, 128 * c:128 * c + 128], (8, 128))

    def u_compute(j, c):
        kw = KR.at[c].bitcast(u32)
        vw = VR.at[c].bitcast(u32)
        taps = [jnp.concatenate([TAP[t, c]] * 2, axis=0) for t in range(4)]
        for nc in range(8):
            n0 = 128 * j + 16 * nc
            b = PADW + 2 * n0
            w0 = kw[pl.ds(b, 16, stride=2), :]
            w1 = kw[pl.ds(b + 1, 16, stride=2), :]
            wm1 = kw[pl.ds(b - 1, 16, stride=2), :]
            wm2 = kw[pl.ds(b - 2, 16, stride=2), :]
            kk = {-3: _hi(wm2), -2: _lo(wm1), -1: _hi(wm1), 0: _lo(w0), 1: _hi(w0), 2: _lo(w1), 3: _hi(w1)}
            v0 = vw[pl.ds(2 * n0, 16, stride=2), :]
            v1 = vw[pl.ds(2 * n0 + 1, 16, stride=2), :]
            vv = [_lo(v0), _hi(v0), _lo(v1), _hi(v1)]
            for r in range(4):
                ks = kk[r] * taps[0] + kk[r - 1] * taps[1] + kk[r - 2] * taps[2] + kk[r - 3] * taps[3]
                UB[r, c, pl.ds(16 * nc, 16), :] = (ks * vv[r]).astype(bf16)

    def k_transpose(j, c):
        xk = SK[pl.ds(128 * c, 128), pl.ds(BLK * j, BLK)].astype(f32)
        TB[c] = xk.T
        for r in range(4):
            KB[r, c] = TB.at[c][pl.ds(r, 128, stride=4), :].astype(bf16)

    def fwd(j, c, src):
        a = []
        for r in range(4):
            lhs = pltpu.bitcast(FS[r], bf16)
            o = _dot(lhs, src[r, c]).reshape(16, 2, 8, 128)
            a.append((o[:, 0], o[:, 1]))
        s02 = (a[0][0] + a[2][0], a[0][1] + a[2][1])
        d02 = (a[0][0] - a[2][0], a[0][1] - a[2][1])
        s13 = (a[1][0] + a[3][0], a[1][1] + a[3][1])
        d13 = (a[1][0] - a[3][0], a[1][1] - a[3][1])
        return [(s02[0] + s13[0], s02[1] + s13[1]),
                (d02[0] + d13[1], d02[1] - d13[0]),
                (s02[0] - s13[0], s02[1] - s13[1]),
                (d02[0] - d13[1], d02[1] + d13[0])]

    def fwd_u(j, c):
        xs = fwd(j, c, UB)
        for q in range(4):
            U[j, q, c, 0] = xs[q][0]
            U[j, q, c, 1] = xs[q][1]

    def fwd_k(m, c):
        xs = fwd(m, c, KB)
        for q in range(4):
            re, im = xs[q]
            if m == 0:
                re = re + TAP[4, c][None]
            if m + 1 < NB:
                KP[m + 1, q, c, 0] = re
                KP[m + 1, q, c, 1] = im
            if m > 0:
                pr = KP[m, q, c, 0]
                pi = KP[m, q, c, 1]
                re = jnp.concatenate([re[:8] - pi[:8], re[8:] + pi[8:]], axis=0)
                im = jnp.concatenate([im[:8] + pr[:8], im[8:] - pr[8:]], axis=0)
            KP[m, q, c, 0] = re
            KP[m, q, c, 1] = im

    def mac(i, c, v0, nv):
        w = []
        for q in range(4):
            ar = ai = None
            for j in range(i + 1):
                ur = U[j, q, c, 0, pl.ds(v0, nv)]
                ui = U[j, q, c, 1, pl.ds(v0, nv)]
                kr = KP[i - j, q, c, 0, pl.ds(v0, nv)]
                ki = KP[i - j, q, c, 1, pl.ds(v0, nv)]
                tr = ur * kr - ui * ki
                ti = ur * ki + ui * kr
                ar = tr if ar is None else ar + tr
                ai = ti if ai is None else ai + ti
            w.append((ar, ai))
        t0 = (w[0][0] + w[2][0], w[0][1] + w[2][1])
        t1 = (w[0][0] - w[2][0], w[0][1] - w[2][1])
        t2 = (w[1][0] + w[3][0], w[1][1] + w[3][1])
        t3 = (w[1][0] - w[3][0], w[1][1] - w[3][1])
        bs = [(t0[0] + t2[0], t0[1] + t2[1]),
              (t1[0] - t3[1], t1[1] + t3[0]),
              (t0[0] - t2[0], t0[1] - t2[1]),
              (t1[0] + t3[1], t1[1] - t3[0])]
        for r in range(4):
            val = jnp.stack([bs[r][0], bs[r][1]], axis=1).reshape(16 * nv, 128)
            BB[r, c, pl.ds(16 * v0, 16 * nv), :] = val.astype(bf16)

    def inv_gate(i, rp):
        xw = [XR.at[c].bitcast(u32)[pl.ds(256 * i + rp, 128, stride=2), :] for c in range(NT)]
        zs = []
        for e in range(2):
            r = 2 * rp + e
            y = _dot(pltpu.bitcast(GS[r], bf16), _cat([BB[r, c] for c in range(NT)]))
            xr = _cat([(_lo if e == 0 else _hi)(w) for w in xw])
            h = xr + _ln(xr) * y
            xb = _ln(h)
            z = _ln(xb)
            for c in range(NT):
                H.at[c][pl.ds(BLK * i + r, 128, stride=4), :] = h[:, 128 * c:128 * c + 128]
                XB.at[c][pl.ds(BLK * i + r, 128, stride=4), :] = xb[:, 128 * c:128 * c + 128]
            zs.append(z.astype(bf16))
        return jnp.concatenate(zs, axis=0)

    def mm1(i, rp, z):
        a = _gelu(_dot(z, wload(W1, 0, D)))
        for e in range(2):
            r = 2 * rp + e
            for c in range(NT):
                A.at[c][pl.ds(APAD + BLK * i + r, 128, stride=4), :] = a[128 * e:128 * e + 128, 128 * c:128 * c + 128]

    lane = lax.broadcasted_iota(i32, (256, 128), 1)

    def c2(cc):
        t0 = 256 * cc

        def ld(c, s):
            return A[c, pl.ds(APAD + t0 + s, 256), :]
        sh = _cat([ld(0, -1),
                   jnp.where(lane < 32, ld(1, -1), ld(1, 1)),
                   jnp.where(lane < 64, ld(2, 1), ld(2, -2)),
                   jnp.where(lane < 96, ld(3, -2), ld(3, 2)),
                   ld(4, 2)]).astype(bf16)
        hs = _dot(sh, wload(W2, 0, D))
        x1 = _cat([XB[c, pl.ds(t0, 256), :] for c in range(NT)]) + hs
        m = _ln(x1).astype(bf16)
        acc = _cat([H[c, pl.ds(t0, 256), :] for c in range(NT)]) + x1
        for c0 in range(0, FF, 256):
            cw = min(256, FF - c0)
            g = _gelu(_dot_nt(m, wload(W3, c0, cw))).astype(bf16)
            acc = acc + _dot(g, wload(W4, c0, cw))
        OUT[pl.ds(t0, 256), :] = acc.astype(bf16)
        cpo = dma(OUT.at[pl.ds(t0, 256), :], o_hbm.at[pl.ds(t0, 256), :])
        cpo.start()
        return cpo

    def c1_front(j):
        wait(('sk', j))
        if j == 0:
            wait('f')
        for c in range(NT):
            k_transpose(j, c)
            fwd_k(j, c)
        wait(('k', j))
        wait(('v', j))
        for c in range(NT):
            u_compute(j, c)
            fwd_u(j, c)

    def c1_back(j):
        for c in range(NT):
            for v0 in range(0, 16, 2):
                mac(j, c, v0, 2)
        if j == 0:
            wait('g')
        wait(('x', j))
        zs = [inv_gate(j, rp) for rp in range(2)]
        if j == 0:
            wait('w1')
        for rp in range(2):
            mm1(j, rp, zs[rp])

    outs = []
    c1_front(0)
    c1_back(0)
    c1_front(1)
    c1_back(1)
    wait('w2')
    wait('w3')
    wait('w4')
    outs.append(c2(0))
    outs.append(c2(1))
    c1_front(2)
    outs.append(c2(2))
    c1_back(2)
    outs.append(c2(3))
    c1_front(3)
    outs.append(c2(4))
    c1_back(3)
    for cc in range(5, 8):
        outs.append(c2(cc))
    for c in outs:
        c.wait()


def _build():
    fw, gw = _dft_constants()
    any_spec = pl.BlockSpec(memory_space=pl.ANY)
    vm = pltpu.VMEM
    scratch = [
        vm((NT, 2 * PADW + S, 128), bf16),
        vm((NT, S, 128), bf16),
        vm((NT, S, 128), bf16),
        vm((D, S), bf16),
        vm((NT, D, 128), bf16),
        vm((NT, D, 128), bf16),
        vm((NT, FF, 128), bf16),
        vm((NT, FF, 128), bf16),
        vm((4, 128, 128), u32),
        vm((4, 64, 256), u32),
        vm((4, D), bf16),
        vm((D,), bf16),
        vm((5, NT, 8, 128), f32),
        vm((NT, BLK, 128), f32),
        vm((4, NT, 128, 128), bf16),
        vm((4, NT, 128, 128), bf16),
        vm((NB, 4, NT, 2, 16, 8, 128), f32),
        vm((NB, 4, NT, 2, 16, 8, 128), f32),
        vm((4, NT, 256, 128), bf16),
        vm((NT, S, 128), f32),
        vm((NT, S, 128), f32),
        vm((NT, S + 2 * APAD, 128), f32),
        vm((S, D), bf16),
        pltpu.SemaphoreType.DMA((128,)),
    ]
    call = pl.pallas_call(
        _kernel,
        out_shape=jax.ShapeDtypeStruct((S, D), bf16),
        in_specs=[any_spec] * 12,
        out_specs=any_spec,
        scratch_shapes=scratch,
        compiler_params=pltpu.CompilerParams(vmem_limit_bytes=110 * 1024 * 1024),
        name="fused_h3_mixer",
    )
    return call, fw, gw


@jax.jit
def pallas_sequential_preLN__ssm_conv_h3__mixer_s_mlp__prompt_kernel(
    A_q, A_k, A_v, A_shift_k, A_ssm_k, A_ssm_D, B_x, B_w1, B_w2, B_w3, B_w4,
):
    call, fw, gw = _build()
    out = call(A_q.reshape(S, D), A_k.reshape(S, D), A_v.reshape(S, D), A_shift_k.T, A_ssm_k, A_ssm_D,
               B_w1, B_w2, B_w3.T, B_w4, fw, gw)
    return out.reshape(1, S, D)
```

```python
import functools

import jax
import jax.numpy as jnp
import numpy as np
import jax.experimental.pallas as pl
import jax.experimental.pallas.tpu as pltpu
from jax import lax

f32, bf16, u32, i32 = jnp.float32, jnp.bfloat16, jnp.uint32, jnp.int32

S, D, FF = 2048, 640, 1728
NT = D // 128
BLK = 512
NB = S // BLK
LFFT = 2 * BLK
PADW = 8
APAD = 8
EPS = 1e-5
NV = (4, 1, 1, 1)
M3, M4 = 128, 128
HN = (64, 16, 16, 16)
GSTART = ('m1', 0, 2)
DYN = ('KPR', 'Q', 'UB', 'BB')
WSTEP = 1
GK = ('T', 'u', 'mac', 'q', 'h')
SKIP = ()
DEPTH = {}


def _bf16_bits(a):
    u = np.ascontiguousarray(a, dtype=np.float32).view(np.uint32).astype(np.uint64)
    r = (u + 0x7FFF + ((u >> 16) & 1)) >> 16
    return (r & 0xFFFF).astype(np.uint32)


def _pack_words(a):
    b = _bf16_bits(a)
    return (b[..., 0::2, :] | (b[..., 1::2, :] << np.uint32(16))).astype(np.uint32)


def _dft_constants():
    k1 = np.zeros((16, 8), np.int64)
    for v in range(16):
        for s in range(8):
            k1[v, s] = 2 * (8 * v + s) if v < 8 else 2 * (8 * (v - 8) + s) + 1
    n1 = np.arange(128)
    fm = np.zeros((4, 256, 128))
    gm = np.zeros((4, 128, 256))
    for r in range(4):
        for v in range(16):
            for s in range(8):
                th = 2 * np.pi * (4 * n1 + r) * (k1[v, s] + 0.5) / LFFT
                fm[r, 16 * v + s] = np.cos(th)
                fm[r, 16 * v + 8 + s] = -np.sin(th)
                gm[r, :, 16 * v + s] = np.cos(th) * (2.0 / LFFT)
                gm[r, :, 16 * v + 8 + s] = -np.sin(th) * (2.0 / LFFT)
    gw = np.concatenate([_pack_words(gm), np.zeros((1, 64, 256), np.uint32)], axis=0)
    return _pack_words(fm), gw


def _dot(a, b):
    return jnp.dot(a, b, preferred_element_type=f32)


def _dot_nt(a, b):
    return lax.dot_general(a, b, (((1,), (1,)), ((), ())), preferred_element_type=f32)


def _lo(w):
    return pltpu.bitcast(w << 16, f32)


def _hi(w):
    return pltpu.bitcast(w & jnp.uint32(0xFFFF0000), f32)


def _ln(x):
    m = jnp.mean(x, axis=-1, keepdims=True)
    d = x - m
    v = jnp.mean(d * d, axis=-1, keepdims=True)
    return d * lax.rsqrt(v + EPS)


C0 = float(np.sqrt(2.0 / np.pi))
C1 = float(np.sqrt(2.0 / np.pi) * 0.044715)


def _gelu(x, half=True):
    inner = x * (C0 + C1 * (x * x))
    hx = 0.5 * x if half else x
    return hx + hx * jnp.tanh(inner)


def _cat(xs):
    return jnp.concatenate(xs, axis=1)


def _kernel(x_hbm, k_hbm, v_hbm, sk_hbm, ssmk_hbm, d_hbm, w1_hbm, w2_hbm, w3_hbm, w4_hbm, f_hbm, g_hbm,
            o_hbm,
            KR, VR, XR, SK, W1, W2, W3, W4, FS, GS, SKS, DS, TAP, TB, UB, KB, U, KP, BB, H, XB, A, OUT,
            Y, Q, Z0, Z1, Z2, Z3, R, MB0, MB1, MB2, MB3, GB0, GB1, ZS, sems):
    MBS = [MB0, MB1, MB2, MB3]
    ZB = [Z0, Z1, Z2, Z3]
    GBS = [GB0, GB1]
    nsem = [0]

    def dma(src, dst):
        i = nsem[0]
        nsem[0] += 1
        return pltpu.make_async_copy(src, dst, sems.at[i])

    def tiles(src, dst, r0, nrows, dr0=None):
        dr0 = r0 if dr0 is None else dr0
        return [dma(src.at[pl.ds(r0, nrows), pl.ds(128 * c, 128)], dst.at[c, pl.ds(dr0, nrows), :]) for c in range(NT)]

    cp = {}
    cp['small'] = [dma(sk_hbm, SKS), dma(d_hbm, DS)]
    cp['f'] = [dma(f_hbm, FS)]
    for j in range(NB):
        if j > 0:
            cp['sk', j] = [dma(ssmk_hbm.at[:, pl.ds(BLK * j, BLK)], SK.at[pl.ds(0, D), pl.ds(BLK * j, BLK)])]
        cp['k', j] = tiles(k_hbm, KR, BLK * j, BLK, 2 * PADW + BLK * j)
        cp['v', j] = tiles(v_hbm, VR, BLK * j, BLK)
        cp['x', j] = tiles(x_hbm, XR, BLK * j, BLK)
    for c in range(NT):
        cp['t0', c] = [dma(ssmk_hbm.at[pl.ds(128 * c, 128), pl.ds(0, BLK)], SK.at[pl.ds(128 * c, 128), pl.ds(0, BLK)]),
                       cp['k', 0][c], cp['v', 0][c]]
    cp['g'] = [dma(g_hbm.at[pl.ds(0, 4)], GS)]
    cp['w1'] = tiles(w1_hbm, W1, 0, D)
    cp['w2'] = tiles(w2_hbm, W2, 0, D)
    cp['w3'] = tiles(w3_hbm, W3, 0, FF)
    cp['w4'] = tiles(w4_hbm, W4, 0, FF)
    cp['z'] = [dma(g_hbm.at[4, pl.ds(0, 8), pl.ds(0, 128)], ZS)]
    started = set()

    def start(*keys):
        for key in keys:
            if key in started:
                continue
            started.add(key)
            for c in cp[key]:
                c.start()

    waited = set()

    def wait(*keys):
        for key in keys:
            if key in waited:
                continue
            waited.add(key)
            for c in cp[key]:
                c.wait()

    start(('t0', 0), 'small', 'z', 'f', *[('t0', c) for c in range(1, NT)], ('x', 0))
    D_ = lambda k: DEPTH.get(k, 0)

    for c in range(NT):
        KR[c, pl.ds(0, 2 * PADW), :] = jnp.zeros((2 * PADW, 128), bf16)
        A[c, pl.ds(0, APAD), :] = jnp.zeros((APAD, 128), f32)
        A[c, pl.ds(APAD + S, APAD), :] = jnp.zeros((APAD, 128), f32)

    def wload(W, r0, nrows):
        return _cat([pltpu.bitcast(W.at[c].bitcast(u32)[pl.ds(r0 // 2, nrows // 2), :], bf16) for c in range(NT)])

    wait('small', 'z')
    off = ZS[0, 0].astype(i32)
    skv = SKS[...].astype(f32)
    dv = DS[...].astype(f32).reshape(1, D)
    for t in range(4):
        for c in range(NT):
            TAP[t, c] = jnp.broadcast_to(skv[t:t + 1, 128 * c:128 * c + 128], (8, 128))
    for c in range(NT):
        TAP[4, c] = jnp.broadcast_to(dv[:, 128 * c:128 * c + 128], (8, 128))

    def gate(kind, val):
        if val is None or not G[0] or kind not in GK:
            return
        if kind == 'T':
            SK.at[pl.ds(D, 16), :].bitcast(u32)[:, 0:128] = pltpu.bitcast(val, u32)
        elif kind == 'u':
            KR.at[0].bitcast(u32)[pl.ds(PADW + S // 2, 8), :] = pltpu.bitcast(val, u32)
        elif kind == 'mac':
            U[NB, 0, 0, 0, 0] = val
        elif kind == 'q':
            XR.at[0].bitcast(u32)[pl.ds(S // 2, 8), :] = pltpu.bitcast(val, u32)
        elif kind == 'h':
            Y[0, pl.ds(512, 8), :] = val

    G = [False]
    doff_ = lambda: off if G[0] else 0
    dy = lambda name: doff_() if name in DYN else 0
    offs_ = [ZS[0, 1 + i].astype(i32) for i in range(NB)]
    offs = lambda i: offs_[i] if G[0] else 0

    def dyn(ref, n):
        return ref.at[pl.ds(pl.multiple_of(doff_(), 8), n), :] if G[0] else ref

    def tok(x):
        return x[0:8, 0:128]

    def u_item(j, c, nc):
        kw = dyn(KR.at[c].bitcast(u32), PADW + S // 2)
        vw = VR.at[c].bitcast(u32)
        taps = [jnp.concatenate([TAP[t, c]] * 2, axis=0) for t in range(4)]
        n0 = 128 * j + 16 * nc
        b = PADW + 2 * n0
        w0 = kw[pl.ds(b, 16, stride=2), :]
        w1 = kw[pl.ds(b + 1, 16, stride=2), :]
        wm1 = kw[pl.ds(b - 1, 16, stride=2), :]
        wm2 = kw[pl.ds(b - 2, 16, stride=2), :]
        kk = {-3: _hi(wm2), -2: _lo(wm1), -1: _hi(wm1), 0: _lo(w0), 1: _hi(w0), 2: _lo(w1), 3: _hi(w1)}
        v0 = vw[pl.ds(2 * n0, 16, stride=2), :]
        v1 = vw[pl.ds(2 * n0 + 1, 16, stride=2), :]
        vv = [_lo(v0), _hi(v0), _lo(v1), _hi(v1)]
        for r in range(4):
            ks = kk[r] * taps[0] + kk[r - 1] * taps[1] + kk[r - 2] * taps[2] + kk[r - 3] * taps[3]
            ur = ks * vv[r]
            UB[r, c, pl.ds(16 * nc, 16), :] = ur.astype(bf16)
        return tok(ur)

    def t_item(j, c, tt):
        ro = pl.multiple_of(128 * c + doff_(), 16) if G[0] else 128 * c
        xk = SK[pl.ds(ro, 128), pl.ds(BLK * j + 128 * tt, 128)].astype(f32)
        xt = xk.T
        TB[c, pl.ds(128 * tt, 128), :] = xt
        for r in range(4):
            kr = TB.at[c][pl.ds(128 * tt + r, 32, stride=4), :]
            KB[r, c, pl.ds(32 * tt, 32), :] = kr.astype(bf16)
        return tok(xt)

    def fwd(src, c):
        a = []
        for r in range(4):
            lhs = pltpu.bitcast(FS[r], bf16)
            o = _dot(lhs, src[r + dy('UB'), c, pl.ds(0, 128), :]).reshape(16, 2, 8, 128)
            a.append((o[:, 0], o[:, 1]))
        s02 = (a[0][0] + a[2][0], a[0][1] + a[2][1])
        d02 = (a[0][0] - a[2][0], a[0][1] - a[2][1])
        s13 = (a[1][0] + a[3][0], a[1][1] + a[3][1])
        d13 = (a[1][0] - a[3][0], a[1][1] - a[3][1])
        return [(s02[0] + s13[0], s02[1] + s13[1]),
                (d02[0] + d13[1], d02[1] - d13[0]),
                (s02[0] - s13[0], s02[1] - s13[1]),
                (d02[0] - d13[1], d02[1] + d13[0])]

    def fu_piece(j, c):
        xs = fwd(UB, c)
        for q in range(4):
            U[j, q, c, pl.ds(0, 16), 0] = xs[q][0]
            U[j, q, c, pl.ds(0, 16), 1] = xs[q][1]
        return xs[3][1].reshape(128, 128)

    def fk_piece(m, c):
        xs = fwd(KB, c)
        for q in range(4):
            re, im = xs[q]
            if m == 0:
                re = re + TAP[4, c][None]
            if m + 1 < NB:
                KP[m + 1, q, c, pl.ds(1, 16), 0] = re
                KP[m + 1, q, c, pl.ds(1, 16), 1] = im
            if m > 0:
                pr = KP[m + dy('KPR'), q, c, pl.ds(1, 16), 0]
                pi = KP[m + dy('KPR'), q, c, pl.ds(1, 16), 1]
                re = jnp.concatenate([re[:8] - pi[:8], re[8:] + pi[8:]], axis=0)
                im = jnp.concatenate([im[:8] + pr[:8], im[8:] - pr[8:]], axis=0)
            KP[m, q, c, pl.ds(1, 16), 0] = re
            KP[m, q, c, pl.ds(1, 16), 1] = im
        return xs[3][1].reshape(128, 128)

    def mac_item(i, c, v0, nv):
        w = []
        for q in range(4):
            ar = ai = None
            for j in range(i + 1):
                ur = U[j + offs(i), q, c, pl.ds(v0, nv), 0]
                ui = U[j + offs(i), q, c, pl.ds(v0, nv), 1]
                kr = KP[i - j + offs(i), q, c, pl.ds(v0 + 1, nv), 0]
                ki = KP[i - j + offs(i), q, c, pl.ds(v0 + 1, nv), 1]
                tr = ur * kr - ui * ki
                ti = ur * ki + ui * kr
                ar = tr if ar is None else ar + tr
                ai = ti if ai is None else ai + ti
            w.append((ar, ai))
        t0 = (w[0][0] + w[2][0], w[0][1] + w[2][1])
        t1 = (w[0][0] - w[2][0], w[0][1] - w[2][1])
        t2 = (w[1][0] + w[3][0], w[1][1] + w[3][1])
        t3 = (w[1][0] - w[3][0], w[1][1] - w[3][1])
        bs = [(t0[0] + t2[0], t0[1] + t2[1]),
              (t1[0] - t3[1], t1[1] + t3[0]),
              (t0[0] - t2[0], t0[1] - t2[1]),
              (t1[0] + t3[1], t1[1] - t3[0])]
        for r in range(4):
            val = jnp.stack([bs[r][0], bs[r][1]], axis=1).reshape(16 * nv, 128)
            BB[r, c, pl.ds(16 * v0, 16 * nv), :] = val.astype(bf16)
        return bs[3][1][nv - 1]

    def q_item(i, r, n0, nn):
        xw = [dyn(XR.at[c].bitcast(u32), S // 2)[pl.ds(256 * i + 2 * n0 + r // 2, nn, stride=2), :] for c in range(NT)]
        q = _ln(_cat([(_hi if r % 2 else _lo)(w) for w in xw]))
        for c in range(NT):
            Q[c, pl.ds(128 * r + n0, nn), :] = q[:, 128 * c:128 * c + 128]
        return tok(q)

    def inv_piece(i, r):
        y = _dot(pltpu.bitcast(GS[r], bf16), _cat([BB[r + dy('BB'), c, pl.ds(0, 256), :] for c in range(NT)]))
        for c in range(NT):
            Y[c, pl.ds(128 * r, 128), :] = y[:, 128 * c:128 * c + 128]
        return y

    def h_item(i, r, n0, nn):
        xw = [XR.at[c].bitcast(u32)[pl.ds(256 * i + 2 * n0 + r // 2, nn, stride=2), :] for c in range(NT)]
        ro = 128 * r + n0
        rd = pl.multiple_of(ro + doff_(), 8) if G[0] else ro
        xr = _cat([(_hi if r % 2 else _lo)(w) for w in xw])
        y = _cat([Y[c, pl.ds(rd, nn), :] for c in range(NT)])
        q = _cat([Q[c + dy('Q'), pl.ds(ro, nn), :] for c in range(NT)])
        h = xr + q * y
        xb = _ln(h)
        zf = _ln(xb)
        z = zf.astype(bf16)
        for c in range(NT):
            H.at[c][pl.ds(BLK * i + 4 * n0 + r, nn, stride=4), :] = h[:, 128 * c:128 * c + 128]
            XB.at[c][pl.ds(BLK * i + 4 * n0 + r, nn, stride=4), :] = xb[:, 128 * c:128 * c + 128]
            ZB[r][c, pl.ds(n0, nn), :] = z[:, 128 * c:128 * c + 128]
        return tok(zf)

    def mm1_sub(i, r):
        z = _cat([ZB[r][c + dy('Z'), pl.ds(0, 128), :] for c in range(NT)])
        pre = _dot(z, wload(W1, 0, D))
        a = _gelu(pre)
        for c in range(NT):
            A.at[c][pl.ds(APAD + BLK * i + r, 128, stride=4), :] = a[:, 128 * c:128 * c + 128]
        return pre

    lane = lax.broadcasted_iota(i32, (128, 128), 1)

    def mm2_sub(cc, k):
        t0 = 256 * cc + 128 * k

        def ld(c, s):
            return A[c, pl.ds(APAD + t0 + s, 128), :]
        sh = _cat([ld(0, -1),
                   jnp.where(lane < 32, ld(1, -1), ld(1, 1)),
                   jnp.where(lane < 64, ld(2, 1), ld(2, -2)),
                   jnp.where(lane < 96, ld(3, -2), ld(3, 2)),
                   ld(4, 2)]).astype(bf16)
        hs = _dot(sh, wload(W2, 0, D))
        x1 = _cat([XB[c + doff_(), pl.ds(t0, 128), :] for c in range(NT)]) + hs
        m = _ln(x1).astype(bf16)
        for c in range(NT):
            R[c, pl.ds(t0, 128), :] = H[c + doff_(), pl.ds(t0, 128), :] + x1[:, 128 * c:128 * c + 128]
            MBS[(2 * cc + k) % 4][c, pl.ds(0, 128), :] = m[:, 128 * c:128 * c + 128]
        return hs

    def mm3_sub(cc, k):
        pres = []
        for r0 in range(0, 128, M3):
            m = _cat([MBS[(2 * cc + k) % 4][c + dy('MB'), pl.ds(r0, M3), :] for c in range(NT)])
            pre = _dot_nt(m, wload(W3, 0, FF))
            g = _gelu(pre, half=False).astype(bf16)
            for kt in range(14):
                cw = min(128, FF - 128 * kt)
                GBS[k][kt, pl.ds(r0, M3), pl.ds(0, cw)] = g[:, 128 * kt:128 * kt + cw]
            pres.append(pre)
        return pres

    outs = []

    def mm4_sub(cc, k):
        t0 = 256 * cc + 128 * k
        hs = []
        for r0 in range(0, 128, M4):
            g = _cat([GBS[k][kt + dy('GB'), pl.ds(r0, M4), pl.ds(0, min(128, FF - 128 * kt))] for kt in range(14)])
            h2 = _dot(g, wload(W4, 0, FF))
            res = _cat([R[c + dy('H'), pl.ds(t0 + r0, M4), :] for c in range(NT)]) + 0.5 * h2
            OUT[pl.ds(t0 + r0, M4), :] = res.astype(bf16)
            hs.append(h2)
        cpo = dma(OUT.at[pl.ds(t0, 128), :], o_hbm.at[pl.ds(t0, 128), :])
        cpo.start()
        outs.append(cpo)
        return hs

    def slots_of(src):
        sl = []
        for s_ in (src if isinstance(src, list) else [src]):
            rows, cols = s_.shape
            sl += [s_[rr:rr + 8, 128 * ct:128 * ct + 128] for ct in range(cols // 128) for rr in range(0, rows, 8)]
        return sl

    def host(items, src=None, clock=None, depth=0, period=1):
        sl = slots_of(src) if src is not None else None
        if src is not None:
            items = [it for it in items if it[0] not in SKIP]
        n = len(items)
        toks = []
        for qi, (kind, fn) in enumerate(items):
            deps = []
            if sl is not None:
                deps.append(sl[(qi * len(sl)) // n])
            if clock is not None:
                deps.append(clock)
                for _ in range(period):
                    clock = pltpu.roll(clock, 1, 1)
            if depth and qi >= depth:
                deps.append(toks[qi - depth])
            val = None
            for d_ in deps:
                val = d_ if val is None else val + d_
            gate(kind, val)
            toks.append(fn())
        return toks[-1] if toks else None

    P = functools.partial
    t_items = lambda j: [('T', P(t_item, j, c, tt)) for c in range(NT) for tt in range(4)]
    u_items = lambda j: [('u', P(u_item, j, c, nc)) for c in range(NT) for nc in range(8)]
    mac_items = lambda i: [('mac', P(mac_item, i, c, v0, NV[i])) for c in range(NT) for v0 in range(0, 16, NV[i])]
    q_items = lambda i: [('q', P(q_item, i, r, n0, HN[i])) for r in range(4) for n0 in range(0, 128, HN[i])]
    h_items = lambda i: [('h', P(h_item, i, r, n0, HN[i])) for r in range(4) for n0 in range(0, 128, HN[i])]

    def merge(*lists):
        tagged = []
        for l in lists:
            n = len(l)
            tagged += [((k + 0.5) / n, x) for k, x in enumerate(l)]
        tagged.sort(key=lambda t: t[0])
        return [x for _, x in tagged]

    seq = []

    def add(name, units, fn):
        seq.append((name, units, fn))

    def act(fn):
        seq.append((None, 0, fn))

    def K_(j, *cs):
        for c in cs:
            add(('fk', j, c), 8, P(fk_piece, j, c))

    def U_(j, *cs):
        for c in cs:
            add(('fu', j, c), 8, P(fu_piece, j, c))

    def I_(j, *rs):
        for r in rs:
            add(('inv', j, r), 10, P(inv_piece, j, r))

    def M1(j, *rs):
        for r in rs:
            add(('m1', j, r), 25, P(mm1_sub, j, r))

    def M2(*cks):
        for cc, k in cks:
            add(('m2', cc, k), 25, P(mm2_sub, cc, k))

    def M3_(cc, k):
        add(('m3', cc, k), 70, P(mm3_sub, cc, k))

    def M4_(cc, k):
        add(('m4', cc, k), 70, P(mm4_sub, cc, k))

    W_ = lambda *k: act(P(wait, *k))
    S_ = lambda *k: act(P(start, *k))
    R5 = range(NT)
    groups = []

    def G_(items, a, b=None, f0=0.0, f1=1.0):
        groups.append(([it for it in items if it[0] not in SKIP], a, b or a, f0, f1))

    bysplit = lambda items, n: [items[len(items) * i // n: len(items) * (i + 1) // n] for i in range(n)]
    t0_, u0_, m0 = bysplit(t_items(0), 5), bysplit(u_items(0), 5), bysplit(mac_items(0), 5)
    q0 = bysplit(q_items(0), 4)
    for c in R5:
        if c % WSTEP == 0:
            W_(*[('t0', c2) for c2 in range(c, min(c + WSTEP, NT))])
        if c == 0:
            W_('f')
        if c == 1:
            S_('g', ('sk', 1), 'w1', ('k', 1), ('v', 1))
        act(P(host, t0_[c]))
        act(P(host, u0_[c]))
        K_(0, c)
        U_(0, c)
        act(P(host, m0[c]))
    W_(('x', 0))
    act(P(host, q0[0] + q0[1]))
    S_('w2', ('x', 1), 'w3')
    W_('g', ('sk', 1))
    h0 = bysplit(h_items(0), 4)
    I_(0, 0, 1)
    G_(q0[2] + q0[3], ('inv', 0, 0), ('inv', 0, 1))
    I_(0, 2, 3)
    G_(h0[0], ('inv', 0, 2), ('inv', 0, 3))
    G_(t_items(1), ('inv', 0, 1), ('inv', 0, 3))
    K_(1, 0, 1)
    G_(h0[1], ('fk', 1, 0), ('fk', 1, 1))
    W_('w1')
    M1(0, 0)
    G_(h0[2], ('m1', 0, 0), f1=0.6)
    K_(1, 2)
    M1(0, 1)
    G_(h0[3], ('m1', 0, 1), f1=0.6)
    K_(1, 3, 4)
    W_(('k', 1), ('v', 1))
    M1(0, 2, 3)
    G_(u_items(1), ('m1', 0, 2), ('m1', 0, 3), f1=0.6)
    U_(1, *R5)
    W_(('x', 1))
    S_('w4')
    W_('w2')
    M2((0, 0), (0, 1))
    G_(mac_items(1), ('fu', 1, 2), ('m2', 0, 1), f1=0.6)
    S_(('sk', 2), ('x', 2), ('k', 2), ('v', 2))
    I_(1, 0, 1, 2, 3)
    G_(q_items(1), ('inv', 1, 0), ('inv', 1, 3))
    W_('w3')
    M3_(0, 0)
    M3_(0, 1)
    h1 = bysplit(h_items(1), 4)
    G_(h1[0] + h1[1], ('m3', 0, 0), f1=0.8)
    G_(h1[2] + h1[3], ('m3', 0, 0), ('m3', 0, 1), f0=0.8, f1=0.6)
    M1(1, 0, 1, 2, 3)
    W_('w4')
    M4_(0, 0)
    W_(('sk', 2), ('x', 2))
    S_(('sk', 3), ('x', 3), ('k', 3), ('v', 3))
    M2((1, 0))
    M4_(0, 1)
    G_(t_items(2), ('m4', 0, 1), f1=0.7)
    M2((1, 1))
    W_(('k', 2), ('v', 2))
    M3_(1, 0)
    K_(2, 0)
    M3_(1, 1)
    K_(2, 1)
    M2((2, 0))
    M4_(1, 0)
    G_(u_items(2), ('m3', 1, 0), ('m4', 1, 0), f1=0.5)
    U_(2, 0, 1)
    K_(2, 2)
    M2((2, 1))
    U_(2, 2, 3)
    K_(2, 3)
    M4_(1, 1)
    U_(2, 4)
    K_(2, 4)
    M3_(2, 0)
    M3_(2, 1)
    mc = bysplit(mac_items(2), 5)
    G_(mc[0] + mc[1], ('m4', 1, 1), f0=0.0)
    G_(mc[2] + mc[3] + mc[4], ('m3', 2, 0), ('m3', 2, 1), f1=0.6)
    G_(q_items(2), ('m2', 2, 1), ('m4', 1, 1), f1=0.5)
    I_(2, 0, 1)
    M2((3, 0))
    W_(('sk', 3), ('x', 3), ('k', 3), ('v', 3))
    M4_(2, 0)
    I_(2, 2, 3)
    M4_(2, 1)
    M1(2, 0, 1)
    M3_(3, 0)
    M1(2, 2, 3)
    h2_ = bysplit(h_items(2), 2)
    G_(h2_[0], ('m4', 2, 0), f1=0.9)
    G_(h2_[1], ('m4', 2, 1), f1=0.7)
    M4_(3, 0)
    G_(t_items(3), ('m3', 3, 0), ('m4', 3, 0), f0=0.3, f1=0.4)
    G_(q_items(3), ('m4', 3, 0), ('m2', 4, 0), f0=0.3)
    M2((3, 1))
    K_(3, 0)
    M2((4, 0))
    K_(3, 1)
    M3_(3, 1)
    K_(3, 2)
    M2((4, 1))
    K_(3, 3)
    M4_(3, 1)
    K_(3, 4)
    G_(u_items(3), ('m3', 3, 1), ('m4', 3, 1), f1=0.6)
    U_(3, 0, 1, 2)
    M3_(4, 0)
    U_(3, 3, 4)
    M3_(4, 1)
    M4_(4, 0)
    mc = bysplit(mac_items(3), 5)
    G_(mc[0] + mc[1], ('m3', 4, 0), f0=0.05)
    G_(mc[2] + mc[3] + mc[4], ('m3', 4, 1), ('m4', 4, 0), f1=0.5)
    M2((5, 0))
    I_(3, 0, 1)
    M4_(4, 1)
    I_(3, 2, 3)
    M3_(5, 0)
    M1(3, 0, 1)
    M4_(5, 0)
    M1(3, 2, 3)
    h3_ = bysplit(h_items(3), 2)
    G_(h3_[0], ('m4', 4, 1), f0=0.05, f1=0.9)
    G_(h3_[1], ('m3', 5, 0), f0=0.05, f1=0.8)
    M2((5, 1), (6, 0), (6, 1))
    M3_(5, 1)
    M4_(5, 1)
    M2((7, 0))
    M3_(6, 0)
    M3_(6, 1)
    M2((7, 1))
    M4_(6, 0)
    M4_(6, 1)
    M3_(7, 0)
    M3_(7, 1)
    M4_(7, 0)
    M4_(7, 1)

    pos, t = {}, 0
    for name, units, _ in seq:
        if name is not None:
            pos[name] = (t, t + units)
            t += units
    hosted = {}
    for items, a, b, f0, f1 in groups:
        ta = pos[a][0] + f0 * (pos[a][1] - pos[a][0])
        tb = pos[b][0] + f1 * (pos[b][1] - pos[b][0])
        for n_, it in enumerate(items):
            tt = ta + (tb - ta) * (n_ + 0.5) / len(items)
            for name, (p0_, p1_) in pos.items():
                if p0_ <= tt < p1_:
                    hosted.setdefault(name, []).append(((tt - p0_) / (p1_ - p0_), it))
                    break
    for name, units, fn in seq:
        if name == GSTART:
            G[0] = True
        out = fn()
        if name in hosted:
            sl = slots_of(out)
            for frac, (kind, f_) in sorted(hosted[name], key=lambda x: x[0]):
                gate(kind, sl[int(frac * len(sl))])
                f_()
    for c in outs:
        c.wait()


def _build(interpret=False):
    fw, gw = _dft_constants()
    any_spec = pl.BlockSpec(memory_space=pl.ANY)
    vm = pltpu.VMEM
    scratch = [
        vm((NT, 2 * PADW + S + 32, 128), bf16),
        vm((NT, S + 16, 128), bf16),
        vm((NT, S + 16, 128), bf16),
        vm((D + 16, S), bf16),
        vm((NT, D + 16, 128), bf16),
        vm((NT, D + 16, 128), bf16),
        vm((NT, FF + 16, 128), bf16),
        vm((NT, FF + 16, 128), bf16),
        vm((4, 128, 128), u32),
        vm((4, 64, 256), u32),
        vm((4, D), bf16),
        vm((D,), bf16),
        vm((5, NT, 8, 128), f32),
        vm((NT, BLK + 8, 128), f32),
        vm((4, NT, 128 + 16, 128), bf16),
        vm((4, NT, 128 + 16, 128), bf16),
        vm((NB + 1, 4, NT, 17, 2, 8, 128), f32),
        vm((NB, 4, NT, 17, 2, 8, 128), f32),
        vm((4, NT, 256 + 16, 128), bf16),
        vm((NT, S + 8, 128), f32),
        vm((NT, S + 8, 128), f32),
        vm((NT, S + 3 * APAD, 128), f32),
        vm((S, D), bf16),
        vm((NT, 4 * 128 + 8, 128), f32),
        vm((NT, 4 * 128 + 8, 128), f32),
        vm((NT, 128 + 16, 128), bf16),
        vm((NT, 128 + 16, 128), bf16),
        vm((NT, 128 + 16, 128), bf16),
        vm((NT, 128 + 16, 128), bf16),
        vm((NT, S + 8, 128), f32),
        vm((NT, 128 + 16, 128), bf16),
        vm((NT, 128 + 16, 128), bf16),
        vm((NT, 128 + 16, 128), bf16),
        vm((NT, 128 + 16, 128), bf16),
        vm((14, 128 + 16, 128), bf16),
        vm((14, 128 + 16, 128), bf16),
        pltpu.SMEM((8, 128), u32),
        pltpu.SemaphoreType.DMA((128,)),
    ]
    call = pl.pallas_call(
        _kernel,
        out_shape=jax.ShapeDtypeStruct((S, D), bf16),
        in_specs=[any_spec] * 12,
        out_specs=any_spec,
        scratch_shapes=scratch,
        compiler_params=pltpu.CompilerParams(vmem_limit_bytes=110 * 1024 * 1024),
        name="fused_h3_mixer",
        interpret=interpret,
    )
    return call, fw, gw


@jax.jit
def pallas_sequential_preLN__ssm_conv_h3__mixer_s_mlp__prompt_kernel(
    A_q, A_k, A_v, A_shift_k, A_ssm_k, A_ssm_D, B_x, B_w1, B_w2, B_w3, B_w4,
):
    call, fw, gw = _build()
    out = call(A_q.reshape(S, D), A_k.reshape(S, D), A_v.reshape(S, D), A_shift_k.T, A_ssm_k, A_ssm_D,
               B_w1, B_w2, B_w3.T, B_w4, fw, gw)
    return out.reshape(1, S, D)
```
